```python
import jax
import jax.numpy as jnp

def _softmax(x, axis=-1):
    return jax.nn.softmax(x, axis=axis)
def _gelu(x):
    return jax.nn.gelu(x, approximate=True)
def _silu(x):
    return jax.nn.silu(x)
def _sigmoid(x):
    return jax.nn.sigmoid(x)
def _layernorm(x, axis=-1, eps=1e-5):
    m = jnp.mean(x, axis=axis, keepdims=True)
    v = jnp.var(x, axis=axis, keepdims=True)
    return (x - m) / jnp.sqrt(v + eps)
def _scatter_add(tgt, idx, src, axis=0):
    return tgt.at[idx].add(src)
def _segment_sum(src, seg, n):
    return jax.ops.segment_sum(src, seg, n)
class _Rng:
    def __init__(self, key):
        self._k = key
    def _next(self):
        self._k, sub = jax.random.split(self._k)
        return sub
    def normal(self, shape):
        return jax.random.normal(self._next(), shape, dtype=jnp.bfloat16)
    def randint(self, lo, hi, shape):
        return jax.random.randint(self._next(), shape, lo, hi, dtype=jnp.int32)
    def uniform(self, shape, lo=0.0, hi=1.0):
        return jax.random.uniform(self._next(), shape, jnp.bfloat16, lo, hi)
    def permutation(self, n):
        return jax.random.permutation(self._next(), n)


kernel_name = 'parallel_sum__sliding_block_cached__mixer_s_mlp__decode'

def setup_inputs():
    _rng = _Rng(jax.random.key(int.from_bytes(__import__("os").urandom(4), "little")))
    _w = (lambda a: (lambda t: t.astype(jnp.bfloat16) if jnp.issubdtype(t.dtype, jnp.floating) else t)(jnp.asarray(a)))
    def _A_setup():
        B, Sq, D = 4, 1, 512
        Hq, Hkv, Sk, Dh = 32, 32, 8192, 128
        assert Hq % Hkv == 0, (Hq, Hkv)
        return {
            "x": _w((lambda *s: _rng.normal(s) * 0.05)(B, Sq, D)),
            "k_cache": _w((lambda *s: _rng.normal(s) * 0.05)(B, Hkv, Sk, Dh)),
            "v_cache": _w((lambda *s: _rng.normal(s) * 0.05)(B, Hkv, Sk, Dh)),
            "wq": _w((lambda *s: _rng.normal(s) * 0.05)(D, Hq * Dh) * (D ** -0.5)),
            "wo": _w((lambda *s: _rng.normal(s) * 0.05)(Hq * Dh, D) * ((Hq * Dh) ** -0.5)),
        }
    _A_in = _A_setup()

    def _B_setup():
        B, S, D, F = 4, 1, 512, 1376
        return {
            "x":  _w((lambda *s: _rng.normal(s) * 0.05)(B, S, D)),
            "w1": _w((lambda *s: _rng.normal(s) * 0.05)(D, D) * (D ** -0.5)),
            "w2": _w((lambda *s: _rng.normal(s) * 0.05)(D, D) * (D ** -0.5)),
            "w3": _w((lambda *s: _rng.normal(s) * 0.05)(D, F) * (D ** -0.5)),
            "w4": _w((lambda *s: _rng.normal(s) * 0.05)(F, D) * (F ** -0.5)),
        }
    _B_in = _B_setup()

    return {
        "A_x": _A_in["x"],
        "A_k_cache": _A_in["k_cache"],
        "A_v_cache": _A_in["v_cache"],
        "A_wq": _A_in["wq"],
        "A_wo": _A_in["wo"],
        "B_x": _B_in["x"],
        "B_w1": _B_in["w1"],
        "B_w2": _B_in["w2"],
        "B_w3": _B_in["w3"],
        "B_w4": _B_in["w4"],
    }

def reference(A_x, A_k_cache, A_v_cache, A_wq, A_wo, B_x, B_w1, B_w2, B_w3, B_w4):
    def _A_ref(x, k_cache, v_cache, wq, wo):
        B, Sq, D = x.shape
        Hq, Dh = 32, 128
        Hkv, Sk = k_cache.shape[1], k_cache.shape[2]
        W = min(4096, max(256, Sk // 4))
        rep = Hq // Hkv
        q = (lambda x, *d: x.transpose(*d))((x @ wq).reshape(B, Sq, Hq, Dh), 0, 2, 1, 3)
        k = jnp.repeat(k_cache[:, :, Sk - W:, :], rep, axis=1)
        v = jnp.repeat(v_cache[:, :, Sk - W:, :], rep, axis=1)
        scores = jnp.einsum("bhqd,bhkd->bhqk", q, k) * (Dh ** -0.5)
        p = _softmax(scores, axis=-1)
        o = jnp.einsum("bhqk,bhkd->bhqd", p, v)
        return (lambda x, *d: x.transpose(*d))(o, 0, 2, 1, 3).reshape(B, Sq, Hq * Dh) @ wo

    def _B_ref(x, w1, w2, w3, w4):
        B, S, D = x.shape
        h = _gelu(_layernorm(x, axis=-1) @ w1)
        c = D // 4
        g0 = jnp.pad(h[:, :, 0*c:1*c], ((0, 0), (1, 0), (0, 0)))[:, :S, :]
        g1 = jnp.pad(h[:, :, 1*c:2*c], ((0, 0), (0, 1), (0, 0)))[:, 1:, :]
        g2 = jnp.pad(h[:, :, 2*c:3*c], ((0, 0), (2, 0), (0, 0)))[:, :S, :]
        g3 = jnp.pad(h[:, :, 3*c:   ], ((0, 0), (0, 2), (0, 0)))[:, 2:, :]
        hs = jnp.concatenate([g0, g1, g2, g3], axis=-1) @ w2
        x1 = x + hs
        h2 = _gelu(_layernorm(x1, axis=-1) @ w3) @ w4
        return x1 + h2

    x = A_x
    xn = _layernorm(x, axis=-1)
    return x + _A_ref(xn, A_k_cache, A_v_cache, A_wq, A_wo) + _B_ref(xn, B_w1, B_w2, B_w3, B_w4)
```

```python
import functools

import jax
import jax.numpy as jnp
import jax.experimental.pallas as pl
import jax.experimental.pallas.tpu as pltpu

LN_EPS = 1e-5
NSLOT = 4


def _ln(x):
    m = jnp.mean(x, axis=-1, keepdims=True)
    c = x - m
    v = jnp.mean(c * c, axis=-1, keepdims=True)
    return c / jnp.sqrt(v + LN_EPS)


def _kernel(x_hbm, k_hbm, v_hbm, wq_hbm, wo_hbm, w3_hbm, w4_hbm,
            o_ref,
            x_buf, wq_buf, wo_buf, w3_buf, w4_buf, k_buf, v_buf, q_buf, oh_buf,
            sem_w, sem_k, sem_v,
            *, B, H, S, W, Dh, D, F):
    n_chunks = B * H
    f32, bf16 = jnp.float32, jnp.bfloat16

    def kv_copies(i, slot):
        h = i // B
        b = i % B
        kc = pltpu.make_async_copy(k_hbm.at[b, h, pl.ds(S - W, W), :], k_buf.at[slot], sem_k.at[slot])
        vc = pltpu.make_async_copy(v_hbm.at[b, h, pl.ds(S - W, W), :], v_buf.at[slot], sem_v.at[slot])
        return kc, vc

    x_cp = pltpu.make_async_copy(x_hbm, x_buf, sem_w.at[0])
    wq_cp = pltpu.make_async_copy(wq_hbm, wq_buf, sem_w.at[1])
    wo_cp = pltpu.make_async_copy(wo_hbm, wo_buf, sem_w.at[2])
    w3_cp = pltpu.make_async_copy(w3_hbm, w3_buf, sem_w.at[3])
    w4_cp = pltpu.make_async_copy(w4_hbm, w4_buf, sem_w.at[4])

    x_cp.start()
    wq_cp.start()
    kc, vc = kv_copies(0, 0)
    kc.start(); vc.start()
    wo_cp.start()
    for i in range(1, NSLOT):
        kc, vc = kv_copies(i, i)
        kc.start(); vc.start()

    x_cp.wait()
    x4 = x_buf[...].reshape(B, D).astype(f32)
    x = jnp.concatenate([x4, jnp.zeros((8 - B, D), f32)], axis=0)
    xn = _ln(x).astype(bf16)
    wq_cp.wait()
    q = jnp.dot(xn, wq_buf[...], preferred_element_type=f32)
    q = q.astype(bf16)
    for h in range(H):
        q_buf[h] = q[:, h * Dh:(h + 1) * Dh]
    wo_cp.wait()

    scale = Dh ** -0.5
    row = jax.lax.broadcasted_iota(jnp.int32, (8, Dh), 0)

    def head_body(h, acc):
        qh = q_buf[h]
        oh = jnp.zeros((8, Dh), f32)
        for b in range(B):
            i = h * B + b
            slot = b
            kc, vc = kv_copies(i, slot)
            kc.wait()
            s = jax.lax.dot_general(qh, k_buf[slot], (((1,), (1,)), ((), ())),
                                    preferred_element_type=f32) * scale
            m = jnp.max(s, axis=-1, keepdims=True)
            p = jnp.exp(s - m)
            l = jnp.sum(p, axis=-1, keepdims=True)
            vc.wait()
            o = jnp.dot(p.astype(bf16), v_buf[slot], preferred_element_type=f32) / l
            oh = jnp.where(row == b, o, oh)

            @pl.when(i + NSLOT < n_chunks)
            def _():
                kc2, vc2 = kv_copies(i + NSLOT, slot)
                kc2.start(); vc2.start()

            @pl.when(i == n_chunks - NSLOT - 1)
            def _():
                w3_cp.start()
                w4_cp.start()
        w_off = pl.multiple_of(h * Dh, Dh)
        return acc + jnp.dot(oh.astype(bf16), wo_buf[pl.ds(w_off, Dh), :], preferred_element_type=f32)

    attn = jax.lax.fori_loop(0, H, head_body, jnp.zeros((8, D), f32))

    w3_cp.wait()
    h1 = jax.nn.gelu(jnp.dot(xn, w3_buf[...], preferred_element_type=f32), approximate=True)
    w4_cp.wait()
    h2 = jnp.dot(h1.astype(bf16), w4_buf[...], preferred_element_type=f32)
    out = x + attn + xn.astype(f32) + h2
    o_ref[...] = out[:B].reshape(B, 1, D).astype(o_ref.dtype)


@jax.jit
def pallas_parallel_sum__sliding_block_cached__mixer_s_mlp__decode_kernel(
    A_x, A_k_cache, A_v_cache, A_wq, A_wo, B_x, B_w1, B_w2, B_w3, B_w4,
):
    B, Sq, D = A_x.shape
    _, H, S, Dh = A_k_cache.shape
    F = B_w3.shape[1]
    W = min(4096, max(256, S // 4))
    assert Sq == 1 and B == NSLOT
    bf16 = jnp.bfloat16
    kern = functools.partial(_kernel, B=B, H=H, S=S, W=W, Dh=Dh, D=D, F=F)
    any_spec = pl.BlockSpec(memory_space=pl.ANY)
    return pl.pallas_call(
        kern,
        in_specs=[any_spec] * 7,
        out_specs=pl.BlockSpec(memory_space=pltpu.VMEM),
        out_shape=jax.ShapeDtypeStruct((B, Sq, D), A_x.dtype),
        scratch_shapes=[
            pltpu.VMEM((B, Sq, D), bf16),
            pltpu.VMEM((D, H * Dh), bf16),
            pltpu.VMEM((H * Dh, D), bf16),
            pltpu.VMEM((D, F), bf16),
            pltpu.VMEM((F, D), bf16),
            pltpu.VMEM((NSLOT, W, Dh), bf16),
            pltpu.VMEM((NSLOT, W, Dh), bf16),
            pltpu.VMEM((H, 8, Dh), bf16),
            pltpu.VMEM((8, Dh), jnp.float32),
            pltpu.SemaphoreType.DMA((5,)),
            pltpu.SemaphoreType.DMA((NSLOT,)),
            pltpu.SemaphoreType.DMA((NSLOT,)),
        ],
        compiler_params=pltpu.CompilerParams(vmem_limit_bytes=64 * 1024 * 1024),
    )(A_x, A_k_cache, A_v_cache, A_wq, A_wo, B_w3, B_w4)
```

```python
import functools, contextlib

import jax
import jax.numpy as jnp
import jax.experimental.pallas as pl
import jax.experimental.pallas.tpu as pltpu

LN_EPS = 1e-5
f32, bf16 = jnp.float32, jnp.bfloat16
NT = (((1,), (1,)), ((), ()))


def _ln(x):
    m = jnp.mean(x, axis=-1, keepdims=True)
    c = x - m
    v = jnp.mean(c * c, axis=-1, keepdims=True)
    return c / jnp.sqrt(v + LN_EPS)


def _kernel(x_hbm, k_hbm, v_hbm, wq_hbm, wo_hbm, w3_hbm, w4_hbm,
            o_ref,
            x_buf, wq_buf, wo_buf, w3_buf, w4_buf, k_buf, v_buf,
            xn_buf, q_buf, qg_buf, s_buf, p_buf, l_buf, pv_buf, oh_buf, oh0_buf, acc_buf,
            sems,
            *, B, H, S, W, Dh, D, F, cfg):
    G = 8
    R = 16
    WB = W // G
    NW = W // WB
    NPC = WB // R
    NHG = H // G
    NSTEP = NHG * B * NW
    NS = cfg['nslot']
    WR = 32
    PPH = Dh // WR
    QC = G * Dh
    n_mlp = F // WR
    MLP_STEP = cfg.get('mlp_step', 64)
    ns = jax.named_scope if cfg.get('scopes') else (lambda n: contextlib.nullcontext())
    KP, VP = cfg.get('kprio', 1), cfg.get('vprio', 0)
    TAIL = cfg.get('tail', (4, 2, 1, 1))
    HB = sum(TAIL)
    S_X, S_WO, S_W3, S_W4, S_Q, S_K = 0, 1, 2, 3, 4, 8
    S_V = S_K + NS
    S_T = S_V + NS

    def kv_src(ref, u, j):
        g = u // NW
        w = u % NW
        b = g % B
        hg = g // B
        off = S - W + w * WB + j * R
        if not isinstance(off, int):
            off = pl.multiple_of(off, R)
        return ref.at[b, pl.ds(hg * G, G), pl.ds(off, R), :]

    def k_copy(u, j):
        return pltpu.make_async_copy(kv_src(k_hbm, u, j), k_buf.at[u % NS, :, pl.ds(j * R, R), :],
                                     sems.at[S_K + u % NS])

    def v_copy(u, j):
        return pltpu.make_async_copy(kv_src(v_hbm, u, j), v_buf.at[u % NS, :, pl.ds(j * R, R), :],
                                     sems.at[S_V + u % NS])

    def wo_copy(j, sem):
        r = j * WR
        return pltpu.make_async_copy(wo_hbm.at[pl.ds(r, WR), :], wo_buf.at[pl.ds(r, WR), :], sems.at[sem])

    def wq_copy(c, j):
        r, cc = j * 16, c * QC
        if not isinstance(c, int):
            cc = pl.multiple_of(cc, QC)
        if not isinstance(j, int):
            r = pl.multiple_of(r, 16)
        return pltpu.make_async_copy(wq_hbm.at[pl.ds(r, 16), pl.ds(cc, QC)],
                                     wq_buf.at[pl.ds(r, 16), pl.ds(cc, QC)], sems.at[S_Q + c])

    def mlp_copy(j):
        r = pl.multiple_of(j * WR, WR)
        return (pltpu.make_async_copy(w3_hbm.at[pl.ds(r, WR), :], w3_buf.at[pl.ds(r, WR), :], sems.at[S_W3]),
                pltpu.make_async_copy(w4_hbm.at[pl.ds(r, WR), :], w4_buf.at[pl.ds(r, WR), :], sems.at[S_W4]))

    def wait(buf, sem):
        pltpu.make_async_copy(buf, buf, sems.at[sem]).wait()

    n_wo_front = (H - HB) * PPH
    n_wq1_front = NW * NPC - n_wo_front
    assert 0 <= n_wq1_front <= 32 and n_wq1_front % 2 == 0

    def filler(idx):
        if idx < n_wo_front:
            return wo_copy(HB * PPH + idx, S_WO)
        return wq_copy(1, idx - n_wo_front)

    def issue_head(p):
        for j in range(NPC):
            k_copy(p, j).start(priority=KP)
            filler(p * NPC + j).start(priority=VP)

    def issue_pair(p):
        for j in range(NPC):
            k_copy(p, j).start(priority=KP)
            v_copy(p - NW, j).start(priority=VP)

    def issue_v(u):
        for j in range(NPC):
            v_copy(u, j).start(priority=(j % 2 if cfg.get('v3', 'alt') == 'alt' else cfg['v3']))

    def issue_tail():
        h = 0
        for gi, n in enumerate(TAIL):
            for _ in range(n):
                for j in range(PPH):
                    wo_copy(h * PPH + j, S_T + gi).start(priority=(j % 2 if cfg.get('tail_prio') is None else cfg['tail_prio']))
                h += 1

    pltpu.make_async_copy(x_hbm, x_buf, sems.at[S_X]).start(priority=0)
    for j in range(32):
        wq_copy(0, j).start(priority=j % 2)
    for p in range(NS):
        issue_head(p)

    with ns('wait_x'):
        wait(x_buf, S_X)
    x4 = x_buf[...].astype(f32)
    x = jnp.concatenate([x4, jnp.zeros((8 - B, D), f32)], axis=0)
    xn = _ln(x).astype(bf16)
    xn_buf[...] = xn
    acc_buf[...] = x + xn.astype(f32)

    scale = Dh ** -0.5
    row = jax.lax.broadcasted_iota(jnp.int32, (8, Dh), 0)

    def when(cond):
        if isinstance(cond, bool):
            return (lambda f: f()) if cond else (lambda f: None)
        return pl.when(cond)

    def k_part(p):
        g = p // NW
        w = p % NW
        b = g % B
        hg = g // B

        @when(w == 0)
        def _():
            @when(b == 0)
            def _():
                cc = hg * QC if isinstance(hg, int) else pl.multiple_of(hg * QC, QC)
                with ns('wait_wq'):
                    wait(wq_buf.at[:, pl.ds(cc, QC)], S_Q + hg)
                q_buf[...] = jnp.dot(xn_buf[...], wq_buf[:, pl.ds(cc, QC)], preferred_element_type=f32)
            qg = jnp.zeros((8, Dh), f32)
            rowq = jax.lax.broadcasted_iota(jnp.int32, (8, QC), 0)
            qb = jnp.sum(jnp.where(rowq == b, q_buf[...], 0.0), axis=0, keepdims=True)
            for j in range(G):
                qg = jnp.where(row == j, jnp.broadcast_to(qb[:, j * Dh:(j + 1) * Dh], (8, Dh)), qg)
            qg_buf[...] = qg.astype(bf16)

        slot = p % NS
        with ns('wait_k'):
            wait(k_buf.at[slot], S_K + slot)
        qg = qg_buf[...]
        row2 = jax.lax.broadcasted_iota(jnp.int32, (8, WB), 0)
        s = jnp.zeros((8, WB), f32)
        for j in range(G):
            sj = jax.lax.dot_general(qg, k_buf[slot, j], NT, preferred_element_type=f32)
            s = jnp.where(row2 == j, sj, s)
        s_buf[w] = s * scale

        @when(w == NW - 1)
        def _():
            s = s_buf[...]
            m = jnp.max(jnp.max(s, axis=0), axis=-1, keepdims=True)
            e = jnp.exp(s - m[None])
            p_buf[...] = e.astype(bf16)
            l = jnp.sum(jnp.sum(e, axis=0), axis=-1, keepdims=True)
            l_buf[...] = jnp.broadcast_to(l, (8, Dh))

    def v_part(u):
        g = u // NW
        w = u % NW
        b = g % B
        hg = g // B
        slot = u % NS
        with ns('wait_v'):
            wait(v_buf.at[slot], S_V + slot)
        pw = p_buf[w]
        if isinstance(w, int):
            o = jnp.zeros((8, Dh), f32) if w == 0 else pv_buf[...]
        else:
            o = jnp.where(w == 0, jnp.zeros((8, Dh), f32), pv_buf[...])
        for j in range(G):
            oj = jnp.dot(pw, v_buf[slot, j], preferred_element_type=f32)
            o = jnp.where(row == j, o + oj, o)
        pv_buf[...] = o

        @when(w == NW - 1)
        def _():
            og = o / l_buf[...]
            for j in range(G):
                oj = jnp.broadcast_to(og[j:j + 1, :], (8, Dh))
                oh_buf[j] = jnp.where(row == b, oj, oh_buf[j])

            @when(b == B - 1)
            def _():
                with ns('outproj'):
                    @when(hg == 0)
                    def _():
                        wait(wo_buf.at[pl.ds(HB * Dh, (H - HB) * Dh), :], S_WO)
                        for j in range(HB):
                            oh0_buf[j] = oh_buf[j].astype(bf16)
                        if HB < G:
                            a = acc_buf[...]
                            for j in range(HB, G):
                                a = a + jnp.dot(oh_buf[j].astype(bf16), wo_buf[pl.ds(j * Dh, Dh), :],
                                                preferred_element_type=f32)
                            acc_buf[...] = a

                    @when(hg > 0)
                    def _():
                        a = acc_buf[...]
                        for j in range(G):
                            r0 = (hg * G + j) * Dh
                            if not isinstance(r0, int):
                                r0 = pl.multiple_of(r0, Dh)
                            a = a + jnp.dot(oh_buf[j].astype(bf16), wo_buf[pl.ds(r0, Dh), :],
                                            preferred_element_type=f32)
                        acc_buf[...] = a

    pv_buf[...] = jnp.zeros((8, Dh), f32)
    for j in range(G):
        oh_buf[j] = jnp.zeros((8, Dh), f32)

    n_extra = (96 - n_wq1_front) // 2

    def extras(p):
        @when(p < n_extra)
        def _():
            e = n_wq1_front + 2 * p
            wq_copy(1 + e // 32, e % 32).start(priority=0)
            wq_copy(1 + (e + 1) // 32, (e + 1) % 32).start(priority=1)

        @when((p >= 8) & (p < 8 + n_mlp) if not isinstance(p, int) else (8 <= p < 8 + n_mlp))
        def _():
            c3, c4 = mlp_copy(p - 8)
            c3.start(priority=0)
            c4.start(priority=1)

    for p in range(NW):
        k_part(p)
        with ns('issue'):
            extras(p)
            if p + NS < NW:
                issue_head(p + NS)
            else:
                issue_pair(p + NS)

    def step(p, carry):
        v_part(p - NW)
        k_part(p)
        with ns('issue'):
            extras(p)
            pn = p + NS

            @pl.when(pn < NSTEP)
            def _():
                issue_pair(pn)

            @pl.when(pn >= NSTEP)
            def _():
                issue_v(pn - NW)

            if cfg.get('tail_at', NSTEP) < NSTEP - NW:
                @pl.when(p - NW == cfg['tail_at'])
                def _():
                    issue_tail()

        @pl.when(p == MLP_STEP)
        def _():
            with ns('mlp'):
                wait(w3_buf, S_W3)
                h1 = jax.lax.dot_general(xn_buf[...], w3_buf[...], NT, preferred_element_type=f32)
                h1 = jax.nn.gelu(h1, approximate=True)
                wait(w4_buf, S_W4)
                acc_buf[...] += jnp.dot(h1.astype(bf16), w4_buf[...], preferred_element_type=f32)
        return carry

    jax.lax.fori_loop(NW, NSTEP, step, 0)

    for u in range(NSTEP - NW, NSTEP):
        v_part(u)
        if u + NS < NSTEP:
            issue_v(u + NS)
        if u == cfg.get('tail_at', NSTEP - 1 - NS):
            issue_tail()

    a = acc_buf[...]
    h = 0
    for gi, n in enumerate(TAIL):
        with ns('wait_tail'):
            wait(wo_buf.at[pl.ds(h * Dh, n * Dh), :], S_T + gi)
        for _ in range(n):
            a = a + jnp.dot(oh0_buf[h], wo_buf[pl.ds(h * Dh, Dh), :], preferred_element_type=f32)
            h += 1
    o_ref[...] = a[:B].astype(o_ref.dtype)


_CFG = dict(tail=(3, 1), tail_prio=1)
cfg = _CFG
cfg.setdefault('nslot', 4)


@jax.jit
def pallas_parallel_sum__sliding_block_cached__mixer_s_mlp__decode_kernel(A_x, A_k_cache, A_v_cache, A_wq, A_wo, B_x, B_w1, B_w2, B_w3, B_w4):
    B, Sq, D = A_x.shape
    _, H, S, Dh = A_k_cache.shape
    F = B_w3.shape[1]
    W = min(4096, max(256, S // 4))
    NS = cfg['nslot']
    G = 8
    WB = W // G
    ntail = len(cfg.get('tail', (4, 2, 1, 1)))
    kern = functools.partial(_kernel, B=B, H=H, S=S, W=W, Dh=Dh, D=D, F=F, cfg=cfg)
    any_spec = pl.BlockSpec(memory_space=pl.ANY)
    out = pl.pallas_call(
        kern,
        in_specs=[any_spec] * 7,
        out_specs=pl.BlockSpec(memory_space=pltpu.VMEM),
        out_shape=jax.ShapeDtypeStruct((B, D), A_x.dtype),
        scratch_shapes=[
            pltpu.VMEM((B, D), bf16),
            pltpu.VMEM((D, H * Dh), bf16),
            pltpu.VMEM((H * Dh, D), bf16),
            pltpu.VMEM((F, D), bf16),
            pltpu.VMEM((F, D), bf16),
            pltpu.VMEM((NS, G, WB, Dh), bf16),
            pltpu.VMEM((NS, G, WB, Dh), bf16),
            pltpu.VMEM((8, D), bf16),
            pltpu.VMEM((8, G * Dh), f32),
            pltpu.VMEM((8, Dh), bf16),
            pltpu.VMEM((G, 8, WB), f32),
            pltpu.VMEM((G, 8, WB), bf16),
            pltpu.VMEM((8, Dh), f32),
            pltpu.VMEM((8, Dh), f32),
            pltpu.VMEM((G, 8, Dh), f32),
            pltpu.VMEM((G, 8, Dh), bf16),
            pltpu.VMEM((8, D), f32),
            pltpu.SemaphoreType.DMA((8 + 2 * NS + max(ntail, 1),)),
        ],
        compiler_params=pltpu.CompilerParams(vmem_limit_bytes=100 * 1024 * 1024,
                                             disable_bounds_checks=cfg.get('nobc', False)),
    )(A_x.reshape(B, D), A_k_cache, A_v_cache, A_wq, A_wo, B_w3.T, B_w4)
    return out.reshape(B, Sq, D)
```

```python
import functools, contextlib

import jax
import jax.numpy as jnp
import jax.experimental.pallas as pl
import jax.experimental.pallas.tpu as pltpu

LN_EPS = 1e-5
f32, bf16 = jnp.float32, jnp.bfloat16
NT = (((1,), (1,)), ((), ()))


def _ln(x):
    m = jnp.mean(x, axis=-1, keepdims=True)
    c = x - m
    v = jnp.mean(c * c, axis=-1, keepdims=True)
    return c / jnp.sqrt(v + LN_EPS)


def _kernel(x_hbm, k_hbm, v_hbm, wq_hbm, wo_hbm, w3_hbm, w4_hbm,
            o_ref,
            x_buf, wq_buf, wo_buf, w3_buf, w4_buf, k_buf, v_buf,
            xn_buf, xm_buf, q_buf, qg_buf, s_buf, p_buf, l_buf, pv_buf, oh_buf, oh0_buf, acc_buf,
            sems,
            *, B, H, S, W, Dh, D, F, cfg):
    G = 8
    R = 16
    WB = W // G
    NW = W // WB
    NPC = WB // R
    NHG = H // G
    NSTEP = NHG * B * NW
    NS = cfg['nslot']
    WR = 32
    PPH = Dh // WR
    QC = G * Dh
    n_mlp = F // WR
    MLP_STEP = cfg.get('mlp_step', 64)
    ns = jax.named_scope if cfg.get('scopes') else (lambda n: contextlib.nullcontext())
    KP, VP = cfg.get('kprio', 1), cfg.get('vprio', 0)
    TAIL = cfg.get('tail', (3, 1))
    assert sum(TAIL) == NHG
    S_X, S_WO, S_W3, S_W4, S_Q, S_K = 0, 1, 2, 3, 4, 8
    S_V = S_K + NS
    S_T = S_V + NS

    def kv_src(ref, u, j):
        g = u // NW
        w = u % NW
        b = g % B
        hg = g // B
        off = S - W + w * WB + j * R
        if not isinstance(off, int):
            off = pl.multiple_of(off, R)
        return ref.at[b, pl.ds(hg * G, G), pl.ds(off, R), :]

    def k_copy(u, j):
        return pltpu.make_async_copy(kv_src(k_hbm, u, j), k_buf.at[u % NS, :, pl.ds(j * R, R), :],
                                     sems.at[S_K + u % NS])

    def v_copy(u, j):
        return pltpu.make_async_copy(kv_src(v_hbm, u, j), v_buf.at[u % NS, :, pl.ds(j * R, R), :],
                                     sems.at[S_V + u % NS])

    def wo4_copy(e):
        return pltpu.make_async_copy(wo_hbm.at[:, pl.ds(e * 8, 8), :], wo_buf.at[:, pl.ds(e * 8, 8), :], sems.at[S_WO])

    def wo_tail_copy(hg, j, sem):
        r = (G - 1) * Dh + j * WR
        return pltpu.make_async_copy(wo_hbm.at[hg, pl.ds(r, WR), :], wo_buf.at[hg, pl.ds(r, WR), :], sems.at[sem])

    def wq_copy(c, j):
        r, cc = (j // 2) * 8, c * QC + (j % 2) * 512
        if not isinstance(cc, int):
            cc = pl.multiple_of(cc, 512)
        if not isinstance(r, int):
            r = pl.multiple_of(r, 8)
        return pltpu.make_async_copy(wq_hbm.at[:, pl.ds(r, 8), pl.ds(cc, 512)],
                                     wq_buf.at[:, pl.ds(r, 8), pl.ds(cc, 512)], sems.at[S_Q + c])

    def mlp_copy(j):
        r = pl.multiple_of(j * WR, WR)
        return (pltpu.make_async_copy(w3_hbm.at[pl.ds(r, WR), :], w3_buf.at[pl.ds(r, WR), :], sems.at[S_W3]),
                pltpu.make_async_copy(w4_hbm.at[pl.ds(r, WR), :], w4_buf.at[pl.ds(r, WR), :], sems.at[S_W4]))

    def wait(buf, sem):
        pltpu.make_async_copy(buf, buf, sems.at[sem]).wait()

    n_wo_front = (G - 1) * Dh // 8
    n_wq1_front = NW * NPC - n_wo_front
    assert 0 <= n_wq1_front <= 32 and n_wq1_front % 2 == 0

    def filler(idx):
        if idx < n_wo_front:
            return wo4_copy(idx)
        return wq_copy(1, idx - n_wo_front)

    def issue_head(p):
        for j in range(NPC):
            k_copy(p, j).start(priority=KP)
            filler(p * NPC + j).start(priority=VP)

    def issue_pair(p):
        kx = cfg.get('kx', ())
        vx = cfg.get('vx', ())
        for j in range(NPC):
            kp = VP if j in kx else KP
            vp = KP if j in vx else VP
            if cfg.get('vfirst'):
                v_copy(p - NW, j).start(priority=vp)
                k_copy(p, j).start(priority=kp)
            else:
                k_copy(p, j).start(priority=kp)
                v_copy(p - NW, j).start(priority=vp)

    def issue_v(u):
        for j in range(NPC):
            v_copy(u, j).start(priority=(j % 2 if cfg.get('v3', 'alt') == 'alt' else cfg['v3']))

    def issue_tail():
        h = 0
        for gi, n in enumerate(TAIL):
            for _ in range(n):
                for j in range(PPH):
                    wo_tail_copy(h, j, S_T + gi).start(priority=cfg.get('tail_prio', 1))
                h += 1

    pltpu.make_async_copy(x_hbm, x_buf, sems.at[S_X]).start(priority=0)
    for j in range(32):
        wq_copy(0, j).start(priority=j % 2)
    for p in range(NS):
        issue_head(p)

    with ns('wait_x'):
        wait(x_buf, S_X)
    x4 = x_buf[...].astype(f32)
    x = jnp.concatenate([x4, jnp.zeros((8 - B, D), f32)], axis=0)
    xn = _ln(x).astype(bf16)
    xn_buf[...] = xn
    xm_buf[...] = _ln(xn.astype(f32)).astype(bf16)
    acc_buf[...] = x + xn.astype(f32)

    scale = Dh ** -0.5
    row = jax.lax.broadcasted_iota(jnp.int32, (8, Dh), 0)

    def when(cond):
        if isinstance(cond, bool):
            return (lambda f: f()) if cond else (lambda f: None)
        return pl.when(cond)

    def k_part(p):
        g = p // NW
        w = p % NW
        b = g % B
        hg = g // B

        @when(w == 0)
        def _():
            @when(b == 0)
            def _():
                cc = hg * QC if isinstance(hg, int) else pl.multiple_of(hg * QC, QC)
                with ns('wait_wq'):
                    wait(wq_buf.at[:, :, pl.ds(cc, QC)], S_Q + hg)
                wqb = wq_buf[:, :, pl.ds(cc, QC)].reshape(D, QC)
                q_buf[...] = jnp.dot(xn_buf[...], wqb, preferred_element_type=f32)
            qg = jnp.zeros((8, Dh), f32)
            rowq = jax.lax.broadcasted_iota(jnp.int32, (8, QC), 0)
            qb = jnp.sum(jnp.where(rowq == b, q_buf[...], 0.0), axis=0, keepdims=True)
            for j in range(G):
                qg = jnp.where(row == j, jnp.broadcast_to(qb[:, j * Dh:(j + 1) * Dh], (8, Dh)), qg)
            qg_buf[...] = qg.astype(bf16)

        slot = p % NS
        with ns('wait_k'):
            wait(k_buf.at[slot], S_K + slot)
        qg = qg_buf[...]
        row2 = jax.lax.broadcasted_iota(jnp.int32, (8, WB), 0)
        s = jnp.zeros((8, WB), f32)
        for j in range(G):
            sj = jax.lax.dot_general(qg, k_buf[slot, j], NT, preferred_element_type=f32)
            s = jnp.where(row2 == j, sj, s)
        s_buf[w] = s * scale

        @when(w == NW - 1)
        def _():
            s = s_buf[...]
            m = jnp.max(jnp.max(s, axis=0), axis=-1, keepdims=True)
            e = jnp.exp(s - m[None])
            p_buf[...] = e.astype(bf16)
            l = jnp.sum(jnp.sum(e, axis=0), axis=-1, keepdims=True)
            l_buf[...] = jnp.broadcast_to(l, (8, Dh))

    def v_part(u):
        g = u // NW
        w = u % NW
        b = g % B
        hg = g // B
        slot = u % NS
        with ns('wait_v'):
            wait(v_buf.at[slot], S_V + slot)
        pw = p_buf[w]
        if isinstance(w, int):
            o = jnp.zeros((8, Dh), f32) if w == 0 else pv_buf[...]
        else:
            o = jnp.where(w == 0, jnp.zeros((8, Dh), f32), pv_buf[...])
        for j in range(G):
            oj = jnp.dot(pw, v_buf[slot, j], preferred_element_type=f32)
            o = jnp.where(row == j, o + oj, o)
        pv_buf[...] = o

        @when(w == NW - 1)
        def _():
            og = o / l_buf[...]
            for j in range(G):
                oj = jnp.broadcast_to(og[j:j + 1, :], (8, Dh))
                oh_buf[j] = jnp.where(row == b, oj, oh_buf[j])

            @when(b == B - 1)
            def _():
                with ns('outproj'):
                    @when(hg == 0)
                    def _():
                        wait(wo_buf.at[:, pl.ds(0, (G - 1) * Dh), :], S_WO)
                    oh0_buf[hg] = oh_buf[G - 1].astype(bf16)
                    a = acc_buf[...]
                    for j in range(G - 1):
                        a = a + jnp.dot(oh_buf[j].astype(bf16), wo_buf[hg, pl.ds(j * Dh, Dh), :],
                                        preferred_element_type=f32)
                    acc_buf[...] = a

    pv_buf[...] = jnp.zeros((8, Dh), f32)
    for j in range(G):
        oh_buf[j] = jnp.zeros((8, Dh), f32)

    n_extra = (96 - n_wq1_front) // 2

    def extras(p):
        @when(p < n_extra)
        def _():
            e = n_wq1_front + 2 * p
            wq_copy(1 + e // 32, e % 32).start(priority=0)
            wq_copy(1 + (e + 1) // 32, (e + 1) % 32).start(priority=1)

        if not cfg.get('no_mlp'):
            @when((p >= 8) & (p < 8 + n_mlp) if not isinstance(p, int) else (8 <= p < 8 + n_mlp))
            def _():
                c3, c4 = mlp_copy(p - 8)
                c3.start(priority=cfg.get('mlp_prio', (0, 1))[0])
                c4.start(priority=cfg.get('mlp_prio', (0, 1))[1])

    for p in range(NW):
        k_part(p)
        with ns('issue'):
            extras(p)
            if p + NS < NW:
                issue_head(p + NS)
            else:
                issue_pair(p + NS)

    def step(p, carry):
        v_part(p - NW)
        k_part(p)
        with ns('issue'):
            extras(p)
            pn = p + NS

            @pl.when(pn < NSTEP)
            def _():
                issue_pair(pn)

            @pl.when(pn >= NSTEP)
            def _():
                issue_v(pn - NW)

            if cfg.get('tail_at', NSTEP) < NSTEP - NW:
                @pl.when(p - NW == cfg['tail_at'])
                def _():
                    issue_tail()

        @pl.when(p == (MLP_STEP if not cfg.get('no_mlp') else -1))
        def _():
            with ns('mlp'):
                wait(w3_buf, S_W3)
                h1 = jax.lax.dot_general(xm_buf[...], w3_buf[...], NT, preferred_element_type=f32)
                h1 = jax.nn.gelu(h1, approximate=True)
                wait(w4_buf, S_W4)
                acc_buf[...] += jnp.dot(h1.astype(bf16), w4_buf[...], preferred_element_type=f32)
        return carry

    jax.lax.fori_loop(NW, NSTEP, step, 0)

    for u in range(NSTEP - NW, NSTEP):
        v_part(u)
        if u + NS < NSTEP:
            issue_v(u + NS)
        if u == cfg.get('tail_at', NSTEP - 1 - NS):
            issue_tail()

    a = acc_buf[...]
    h = 0
    for gi, n in enumerate(TAIL):
        with ns('wait_tail'):
            wait(wo_buf.at[pl.ds(h, n), pl.ds((G - 1) * Dh, Dh), :], S_T + gi)
        for _ in range(n):
            a = a + jnp.dot(oh0_buf[h], wo_buf[h, pl.ds((G - 1) * Dh, Dh), :], preferred_element_type=f32)
            h += 1
    o_ref[...] = a[:B].astype(o_ref.dtype)


_CFG = dict(nosc=True, vfirst=True, nslot=5)
cfg = _CFG
cfg.setdefault('nslot', 4)


@jax.jit
def pallas_parallel_sum__sliding_block_cached__mixer_s_mlp__decode_kernel(A_x, A_k_cache, A_v_cache, A_wq, A_wo, B_x, B_w1, B_w2, B_w3, B_w4):
    B, Sq, D = A_x.shape
    _, H, S, Dh = A_k_cache.shape
    F = B_w3.shape[1]
    W = min(4096, max(256, S // 4))
    NS = cfg['nslot']
    G = 8
    WB = W // G
    ntail = len(cfg.get('tail', (3, 1)))
    kern = functools.partial(_kernel, B=B, H=H, S=S, W=W, Dh=Dh, D=D, F=F, cfg=cfg)
    any_spec = pl.BlockSpec(memory_space=pl.ANY)
    out = pl.pallas_call(
        kern,
        in_specs=[any_spec] * 7,
        out_specs=pl.BlockSpec(memory_space=pltpu.VMEM),
        out_shape=jax.ShapeDtypeStruct((B, D), A_x.dtype),
        scratch_shapes=[
            pltpu.VMEM((B, D), bf16),
            pltpu.VMEM((4, D // 4, H * Dh), bf16),
            pltpu.VMEM((H // G, G * Dh, D), bf16),
            pltpu.VMEM((F, D), bf16),
            pltpu.VMEM((F, D), bf16),
            pltpu.VMEM((NS, G, WB, Dh), bf16),
            pltpu.VMEM((NS, G, WB, Dh), bf16),
            pltpu.VMEM((8, D), bf16),
            pltpu.VMEM((8, D), bf16),
            pltpu.VMEM((8, G * Dh), f32),
            pltpu.VMEM((8, Dh), bf16),
            pltpu.VMEM((G, 8, WB), f32),
            pltpu.VMEM((G, 8, WB), bf16),
            pltpu.VMEM((8, Dh), f32),
            pltpu.VMEM((8, Dh), f32),
            pltpu.VMEM((G, 8, Dh), f32),
            pltpu.VMEM((H // G, 8, Dh), bf16),
            pltpu.VMEM((8, D), f32),
            pltpu.SemaphoreType.DMA((8 + 2 * NS + max(ntail, 1),)),
        ],
        compiler_params=pltpu.CompilerParams(vmem_limit_bytes=100 * 1024 * 1024,
                                             disable_bounds_checks=cfg.get('nobc', False),
                                             disable_semaphore_checks=cfg.get('nosc', False),
                                             skip_device_barrier=cfg.get('nobar', False)),
    )(A_x.reshape(B, D), A_k_cache, A_v_cache, A_wq.reshape(4, D // 4, H * Dh),
      A_wo.reshape(H // G, G * Dh, D), B_w3.T, B_w4)
    return out.reshape(B, Sq, D)
```

```python
import functools

import jax
import jax.numpy as jnp
import jax.experimental.pallas as pl
import jax.experimental.pallas.tpu as pltpu

LN_EPS = 1e-5
F32, BF16 = jnp.float32, jnp.bfloat16
NT = (((1,), (1,)), ((), ()))

G = 8
R = 16
NS = 5
WR = 32
KP, VP = 1, 0
TAIL = (3, 1)
MLP_STEP = 64


def _ln(x):
    m = jnp.mean(x, axis=-1, keepdims=True)
    c = x - m
    v = jnp.mean(c * c, axis=-1, keepdims=True)
    return c / jnp.sqrt(v + LN_EPS)


def _when(cond):
    if isinstance(cond, bool):
        return (lambda f: f()) if cond else (lambda f: None)
    return pl.when(cond)


def _mult(x, m):
    return x if isinstance(x, int) else pl.multiple_of(x, m)


def _kernel(x_hbm, k_hbm, v_hbm, wq_hbm, wo_hbm, w3_hbm, w4_hbm,
            o_ref,
            x_buf, wq_buf, wo_buf, w3_buf, w4_buf, k_buf, v_buf,
            xn_buf, xm_buf, q_buf, qg_buf, s_buf, p_buf, l_buf, pv_buf, oh_buf, oh0_buf, acc_buf,
            sems,
            *, B, H, S, W, Dh, D, F):
    WB = W // G
    NW = W // WB
    NPC = WB // R
    NHG = H // G
    NSTEP = NHG * B * NW
    PPH = Dh // WR
    QC = G * Dh
    NQP = (D // 4 // 8) * (QC // 512)
    n_mlp = F // WR
    S_X, S_WO, S_W3, S_W4, S_Q = 0, 1, 2, 3, 4
    S_K = S_Q + NHG
    S_V = S_K + NS
    S_T = S_V + NS

    def kv_src(ref, u, j):
        g = u // NW
        off = _mult(S - W + (u % NW) * WB + j * R, R)
        return ref.at[g % B, pl.ds((g // B) * G, G), pl.ds(off, R), :]

    def k_copy(u, j):
        return pltpu.make_async_copy(kv_src(k_hbm, u, j), k_buf.at[u % NS, :, pl.ds(j * R, R), :],
                                     sems.at[S_K + u % NS])

    def v_copy(u, j):
        return pltpu.make_async_copy(kv_src(v_hbm, u, j), v_buf.at[u % NS, :, pl.ds(j * R, R), :],
                                     sems.at[S_V + u % NS])

    def wo4_copy(e):
        return pltpu.make_async_copy(wo_hbm.at[:, pl.ds(e * 8, 8), :], wo_buf.at[:, pl.ds(e * 8, 8), :],
                                     sems.at[S_WO])

    def wo_tail_copy(hg, j, sem):
        r = (G - 1) * Dh + j * WR
        return pltpu.make_async_copy(wo_hbm.at[hg, pl.ds(r, WR), :], wo_buf.at[hg, pl.ds(r, WR), :],
                                     sems.at[sem])

    def wq_copy(c, j):
        r = _mult((j // 2) * 8, 8)
        cc = _mult(c * QC + (j % 2) * 512, 512)
        return pltpu.make_async_copy(wq_hbm.at[:, pl.ds(r, 8), pl.ds(cc, 512)],
                                     wq_buf.at[:, pl.ds(r, 8), pl.ds(cc, 512)], sems.at[S_Q + c])

    def mlp_copies(j):
        r = _mult(j * WR, WR)
        return (pltpu.make_async_copy(w3_hbm.at[pl.ds(r, WR), :], w3_buf.at[pl.ds(r, WR), :], sems.at[S_W3]),
                pltpu.make_async_copy(w4_hbm.at[pl.ds(r, WR), :], w4_buf.at[pl.ds(r, WR), :], sems.at[S_W4]))

    def wait(buf, sem):
        pltpu.make_async_copy(buf, buf, sems.at[sem]).wait()

    n_wo_front = (G - 1) * Dh // 8
    n_wq1_front = NW * NPC - n_wo_front
    n_extra = ((NHG - 1) * NQP - n_wq1_front) // 2
    assert 0 <= n_wq1_front <= NQP and n_wq1_front % 2 == 0 and sum(TAIL) == NHG

    def issue_head(p):
        for j in range(NPC):
            k_copy(p, j).start(priority=KP)
            e = p * NPC + j
            (wo4_copy(e) if e < n_wo_front else wq_copy(1, e - n_wo_front)).start(priority=VP)

    def issue_pair(p):
        for j in range(NPC):
            v_copy(p - NW, j).start(priority=VP)
            k_copy(p, j).start(priority=KP)

    def issue_v(u):
        for j in range(NPC):
            v_copy(u, j).start(priority=j % 2)

    def issue_tail():
        h = 0
        for gi, n in enumerate(TAIL):
            for _ in range(n):
                for j in range(PPH):
                    wo_tail_copy(h, j, S_T + gi).start(priority=1)
                h += 1

    def issue_extras(p):
        @_when(p < n_extra)
        def _():
            e = n_wq1_front + 2 * p
            wq_copy(1 + e // NQP, e % NQP).start(priority=0)
            wq_copy(1 + (e + 1) // NQP, (e + 1) % NQP).start(priority=1)

        @_when((8 <= p < 8 + n_mlp) if isinstance(p, int) else ((p >= 8) & (p < 8 + n_mlp)))
        def _():
            c3, c4 = mlp_copies(p - 8)
            c3.start(priority=0)
            c4.start(priority=1)

    pltpu.make_async_copy(x_hbm, x_buf, sems.at[S_X]).start(priority=0)
    for j in range(NQP):
        wq_copy(0, j).start(priority=j % 2)
    for p in range(NS):
        issue_head(p)

    wait(x_buf, S_X)
    x = jnp.concatenate([x_buf[...].astype(F32), jnp.zeros((8 - B, D), F32)], axis=0)
    xn = _ln(x).astype(BF16)
    xn_buf[...] = xn
    xm_buf[...] = _ln(xn.astype(F32)).astype(BF16)
    acc_buf[...] = x + xn.astype(F32)
    pv_buf[...] = jnp.zeros((8, Dh), F32)
    for j in range(G):
        oh_buf[j] = jnp.zeros((8, Dh), F32)

    scale = Dh ** -0.5
    row = jax.lax.broadcasted_iota(jnp.int32, (8, Dh), 0)

    def k_part(p):
        g = p // NW
        w = p % NW
        b = g % B
        hg = g // B

        @_when(w == 0)
        def _():
            @_when(b == 0)
            def _():
                cc = _mult(hg * QC, QC)
                wait(wq_buf.at[:, :, pl.ds(cc, QC)], S_Q + hg)
                wq_blk = wq_buf[:, :, pl.ds(cc, QC)].reshape(D, QC)
                q_buf[...] = jnp.dot(xn_buf[...], wq_blk, preferred_element_type=F32)
            rowq = jax.lax.broadcasted_iota(jnp.int32, (8, QC), 0)
            qb = jnp.sum(jnp.where(rowq == b, q_buf[...], 0.0), axis=0, keepdims=True)
            qg = jnp.zeros((8, Dh), F32)
            for j in range(G):
                qg = jnp.where(row == j, jnp.broadcast_to(qb[:, j * Dh:(j + 1) * Dh], (8, Dh)), qg)
            qg_buf[...] = qg.astype(BF16)

        slot = p % NS
        wait(k_buf.at[slot], S_K + slot)
        qg = qg_buf[...]
        row2 = jax.lax.broadcasted_iota(jnp.int32, (8, WB), 0)
        s = jnp.zeros((8, WB), F32)
        for j in range(G):
            sj = jax.lax.dot_general(qg, k_buf[slot, j], NT, preferred_element_type=F32)
            s = jnp.where(row2 == j, sj, s)
        s_buf[w] = s * scale

        @_when(w == NW - 1)
        def _():
            s_all = s_buf[...]
            m = jnp.max(jnp.max(s_all, axis=0), axis=-1, keepdims=True)
            e = jnp.exp(s_all - m[None])
            p_buf[...] = e.astype(BF16)
            l = jnp.sum(jnp.sum(e, axis=0), axis=-1, keepdims=True)
            l_buf[...] = jnp.broadcast_to(l, (8, Dh))

    def v_part(u):
        g = u // NW
        w = u % NW
        b = g % B
        hg = g // B
        slot = u % NS
        wait(v_buf.at[slot], S_V + slot)
        pw = p_buf[w]
        if isinstance(w, int):
            o = jnp.zeros((8, Dh), F32) if w == 0 else pv_buf[...]
        else:
            o = jnp.where(w == 0, jnp.zeros((8, Dh), F32), pv_buf[...])
        for j in range(G):
            oj = jnp.dot(pw, v_buf[slot, j], preferred_element_type=F32)
            o = jnp.where(row == j, o + oj, o)
        pv_buf[...] = o

        @_when(w == NW - 1)
        def _():
            og = o / l_buf[...]
            for j in range(G):
                oj = jnp.broadcast_to(og[j:j + 1, :], (8, Dh))
                oh_buf[j] = jnp.where(row == b, oj, oh_buf[j])

            @_when(b == B - 1)
            def _():
                @_when(hg == 0)
                def _():
                    wait(wo_buf.at[:, pl.ds(0, (G - 1) * Dh), :], S_WO)
                oh0_buf[hg] = oh_buf[G - 1].astype(BF16)
                a = acc_buf[...]
                for j in range(G - 1):
                    a = a + jnp.dot(oh_buf[j].astype(BF16), wo_buf[hg, pl.ds(j * Dh, Dh), :],
                                    preferred_element_type=F32)
                acc_buf[...] = a

    for p in range(NW):
        k_part(p)
        issue_extras(p)
        if p + NS < NW:
            issue_head(p + NS)
        else:
            issue_pair(p + NS)

    def step(p, carry):
        v_part(p - NW)
        k_part(p)
        issue_extras(p)
        pn = p + NS

        @pl.when(pn < NSTEP)
        def _():
            issue_pair(pn)

        @pl.when(pn >= NSTEP)
        def _():
            issue_v(pn - NW)

        @pl.when(p == MLP_STEP)
        def _():
            wait(w3_buf, S_W3)
            h1 = jax.lax.dot_general(xm_buf[...], w3_buf[...], NT, preferred_element_type=F32)
            h1 = jax.nn.gelu(h1, approximate=True)
            wait(w4_buf, S_W4)
            acc_buf[...] += jnp.dot(h1.astype(BF16), w4_buf[...], preferred_element_type=F32)
        return carry

    jax.lax.fori_loop(NW, NSTEP, step, 0)

    for u in range(NSTEP - NW, NSTEP):
        v_part(u)
        if u + NS < NSTEP:
            issue_v(u + NS)
        if u + NS == NSTEP - 1:
            issue_tail()

    a = acc_buf[...]
    h = 0
    for gi, n in enumerate(TAIL):
        wait(wo_buf.at[pl.ds(h, n), pl.ds((G - 1) * Dh, Dh), :], S_T + gi)
        for _ in range(n):
            a = a + jnp.dot(oh0_buf[h], wo_buf[h, pl.ds((G - 1) * Dh, Dh), :], preferred_element_type=F32)
            h += 1
    o_ref[...] = a[:B].astype(o_ref.dtype)


@jax.jit
def pallas_parallel_sum__sliding_block_cached__mixer_s_mlp__decode_kernel(
    A_x, A_k_cache, A_v_cache, A_wq, A_wo, B_x, B_w1, B_w2, B_w3, B_w4,
):
    B, Sq, D = A_x.shape
    _, H, S, Dh = A_k_cache.shape
    F = B_w3.shape[1]
    W = min(4096, max(256, S // 4))
    WB = W // G
    NHG = H // G
    assert Sq == 1 and B <= 8 and A_wq.shape == (D, H * Dh) and H % G == 0
    assert W % (G * R) == 0 and F % WR == 0 and 8 + F // WR <= MLP_STEP < NHG * B * G
    kern = functools.partial(_kernel, B=B, H=H, S=S, W=W, Dh=Dh, D=D, F=F)
    out = pl.pallas_call(
        kern,
        in_specs=[pl.BlockSpec(memory_space=pl.ANY)] * 7,
        out_specs=pl.BlockSpec(memory_space=pltpu.VMEM),
        out_shape=jax.ShapeDtypeStruct((B, D), A_x.dtype),
        scratch_shapes=[
            pltpu.VMEM((B, D), BF16),
            pltpu.VMEM((4, D // 4, H * Dh), BF16),
            pltpu.VMEM((NHG, G * Dh, D), BF16),
            pltpu.VMEM((F, D), BF16),
            pltpu.VMEM((F, D), BF16),
            pltpu.VMEM((NS, G, WB, Dh), BF16),
            pltpu.VMEM((NS, G, WB, Dh), BF16),
            pltpu.VMEM((8, D), BF16),
            pltpu.VMEM((8, D), BF16),
            pltpu.VMEM((8, G * Dh), F32),
            pltpu.VMEM((8, Dh), BF16),
            pltpu.VMEM((G, 8, WB), F32),
            pltpu.VMEM((G, 8, WB), BF16),
            pltpu.VMEM((8, Dh), F32),
            pltpu.VMEM((8, Dh), F32),
            pltpu.VMEM((G, 8, Dh), F32),
            pltpu.VMEM((NHG, 8, Dh), BF16),
            pltpu.VMEM((8, D), F32),
            pltpu.SemaphoreType.DMA((4 + NHG + 2 * NS + len(TAIL),)),
        ],
        compiler_params=pltpu.CompilerParams(vmem_limit_bytes=64 * 1024 * 1024,
                                             disable_semaphore_checks=True),
    )(A_x.reshape(B, D), A_k_cache, A_v_cache, A_wq.reshape(4, D // 4, H * Dh),
      A_wo.reshape(NHG, G * Dh, D), B_w3.T, B_w4)
    return out.reshape(B, Sq, D)
```

```python
import functools

import jax
import jax.numpy as jnp
import jax.experimental.pallas as pl
import jax.experimental.pallas.tpu as pltpu

LN_EPS = 1e-5
F32, BF16 = jnp.float32, jnp.bfloat16
NT = (((1,), (1,)), ((), ()))

G = 8
R = 16
NS = 5
WR = 32
KP, VP = 1, 0
TAIL = (3, 1)
MLP_STEP = 64


def _ln(x):
    m = jnp.mean(x, axis=-1, keepdims=True)
    c = x - m
    v = jnp.mean(c * c, axis=-1, keepdims=True)
    return c / jnp.sqrt(v + LN_EPS)


def _when(cond):
    if isinstance(cond, bool):
        return (lambda f: f()) if cond else (lambda f: None)
    return pl.when(cond)


def _mult(x, m):
    return x if isinstance(x, int) else pl.multiple_of(x, m)


def _kernel(x_hbm, k_hbm, v_hbm, wq_hbm, wo_hbm, w3_hbm, w4_hbm,
            o_ref,
            x_buf, wq_buf, wo_buf, w3_buf, w4_buf, k_buf, v_buf,
            xn_buf, xm_buf, q_buf, qg_buf, s_buf, p_buf, l_buf, pv_buf, oh_buf, oh0_buf, acc_buf,
            sems,
            *, B, H, S, W, Dh, D, F):
    WB = W // G
    NW = W // WB
    NPC = WB // R
    NHG = H // G
    NSTEP = NHG * B * NW
    PPH = Dh // WR
    QC = G * Dh
    NQP = (D // 4 // 8) * (QC // 512)
    n_mlp = F // WR
    S_X, S_WO, S_W3, S_W4, S_Q = 0, 1, 2, 3, 4
    S_K = S_Q + NHG
    NSV = NS + NW
    S_V = S_K + NS
    S_T = S_V + NSV

    def kv_src(ref, u, j):
        g = u // NW
        off = _mult(S - W + (u % NW) * WB + j * R, R)
        return ref.at[g % B, pl.ds((g // B) * G, G), pl.ds(off, R), :]

    def k_copy(u, j):
        return pltpu.make_async_copy(kv_src(k_hbm, u, j), k_buf.at[u % NS, :, pl.ds(j * R, R), :],
                                     sems.at[S_K + u % NS])

    def v_copy(u, j):
        return pltpu.make_async_copy(kv_src(v_hbm, u, j), v_buf.at[u % NSV, :, pl.ds(j * R, R), :],
                                     sems.at[S_V + u % NSV])

    def wo4_copy(e):
        return pltpu.make_async_copy(wo_hbm.at[:, pl.ds(e * 8, 8), :], wo_buf.at[:, pl.ds(e * 8, 8), :],
                                     sems.at[S_WO])

    def wo_tail_copy(hg, j, sem):
        r = (G - 1) * Dh + j * WR
        return pltpu.make_async_copy(wo_hbm.at[hg, pl.ds(r, WR), :], wo_buf.at[hg, pl.ds(r, WR), :],
                                     sems.at[sem])

    def wq_copy(c, j):
        r = _mult((j // 2) * 8, 8)
        cc = _mult(c * QC + (j % 2) * 512, 512)
        return pltpu.make_async_copy(wq_hbm.at[:, pl.ds(r, 8), pl.ds(cc, 512)],
                                     wq_buf.at[:, pl.ds(r, 8), pl.ds(cc, 512)], sems.at[S_Q + c])

    def mlp_copies(j):
        r = _mult(j * WR, WR)
        return (pltpu.make_async_copy(w3_hbm.at[pl.ds(r, WR), :], w3_buf.at[pl.ds(r, WR), :], sems.at[S_W3]),
                pltpu.make_async_copy(w4_hbm.at[pl.ds(r, WR), :], w4_buf.at[pl.ds(r, WR), :], sems.at[S_W4]))

    def wait(buf, sem):
        pltpu.make_async_copy(buf, buf, sems.at[sem]).wait()

    n_wo_front = (G - 1) * Dh // 8
    n_wq1_front = NW * NPC - n_wo_front
    n_extra = ((NHG - 1) * NQP - n_wq1_front) // 2
    assert 0 <= n_wq1_front <= NQP and n_wq1_front % 2 == 0 and sum(TAIL) == NHG

    def issue_head(p):
        for j in range(NPC):
            k_copy(p, j).start(priority=KP)
            e = p * NPC + j
            (wo4_copy(e) if e < n_wo_front else wq_copy(1, e - n_wo_front)).start(priority=VP)

    def issue_pair(p):
        for j in range(NPC):
            v_copy(p - NW, j).start(priority=VP)
            k_copy(p, j).start(priority=KP)

    def issue_vv(u):
        for j in range(NPC):
            v_copy(u, j).start(priority=0)
            v_copy(u + 1, j).start(priority=1)

    def issue_tail():
        h = 0
        for gi, n in enumerate(TAIL):
            for _ in range(n):
                for j in range(PPH):
                    wo_tail_copy(h, j, S_T + gi).start(priority=1)
                h += 1

    def issue_extras(p):
        @_when(p < n_extra)
        def _():
            e = n_wq1_front + 2 * p
            wq_copy(1 + e // NQP, e % NQP).start(priority=0)
            wq_copy(1 + (e + 1) // NQP, (e + 1) % NQP).start(priority=1)

        @_when((8 <= p < 8 + n_mlp) if isinstance(p, int) else ((p >= 8) & (p < 8 + n_mlp)))
        def _():
            c3, c4 = mlp_copies(p - 8)
            c3.start(priority=0)
            c4.start(priority=1)

    pltpu.make_async_copy(x_hbm, x_buf, sems.at[S_X]).start(priority=0)
    for j in range(NQP):
        wq_copy(0, j).start(priority=j % 2)
    for p in range(NS):
        issue_head(p)

    wait(x_buf, S_X)
    x = jnp.concatenate([x_buf[...].astype(F32), jnp.zeros((8 - B, D), F32)], axis=0)
    xn = _ln(x).astype(BF16)
    xn_buf[...] = xn
    xm_buf[...] = _ln(xn.astype(F32)).astype(BF16)
    acc_buf[...] = x + xn.astype(F32)
    pv_buf[...] = jnp.zeros((8, Dh), F32)
    for j in range(G):
        oh_buf[j] = jnp.zeros((8, Dh), F32)

    scale = Dh ** -0.5
    row = jax.lax.broadcasted_iota(jnp.int32, (8, Dh), 0)

    def k_part(p):
        g = p // NW
        w = p % NW
        b = g % B
        hg = g // B

        @_when(w == 0)
        def _():
            @_when(b == 0)
            def _():
                cc = _mult(hg * QC, QC)
                wait(wq_buf.at[:, :, pl.ds(cc, QC)], S_Q + hg)
                wq_blk = wq_buf[:, :, pl.ds(cc, QC)].reshape(D, QC)
                q_buf[...] = jnp.dot(xn_buf[...], wq_blk, preferred_element_type=F32)
            rowq = jax.lax.broadcasted_iota(jnp.int32, (8, QC), 0)
            qb = jnp.sum(jnp.where(rowq == b, q_buf[...], 0.0), axis=0, keepdims=True)
            qg = jnp.zeros((8, Dh), F32)
            for j in range(G):
                qg = jnp.where(row == j, jnp.broadcast_to(qb[:, j * Dh:(j + 1) * Dh], (8, Dh)), qg)
            qg_buf[...] = qg.astype(BF16)

        slot = p % NS
        wait(k_buf.at[slot], S_K + slot)
        qg = qg_buf[...]
        row2 = jax.lax.broadcasted_iota(jnp.int32, (8, WB), 0)
        s = jnp.zeros((8, WB), F32)
        for j in range(G):
            sj = jax.lax.dot_general(qg, k_buf[slot, j], NT, preferred_element_type=F32)
            s = jnp.where(row2 == j, sj, s)
        s_buf[w] = s * scale

        @_when(w == NW - 1)
        def _():
            s_all = s_buf[...]
            m = jnp.max(jnp.max(s_all, axis=0), axis=-1, keepdims=True)
            e = jnp.exp(s_all - m[None])
            p_buf[...] = e.astype(BF16)
            l = jnp.sum(jnp.sum(e, axis=0), axis=-1, keepdims=True)
            l_buf[...] = jnp.broadcast_to(l, (8, Dh))

    def v_part(u):
        g = u // NW
        w = u % NW
        b = g % B
        hg = g // B
        slot = u % NSV
        wait(v_buf.at[slot], S_V + slot)
        pw = p_buf[w]
        if isinstance(w, int):
            o = jnp.zeros((8, Dh), F32) if w == 0 else pv_buf[...]
        else:
            o = jnp.where(w == 0, jnp.zeros((8, Dh), F32), pv_buf[...])
        for j in range(G):
            oj = jnp.dot(pw, v_buf[slot, j], preferred_element_type=F32)
            o = jnp.where(row == j, o + oj, o)
        pv_buf[...] = o

        @_when(w == NW - 1)
        def _():
            og = o / l_buf[...]
            for j in range(G):
                oj = jnp.broadcast_to(og[j:j + 1, :], (8, Dh))
                oh_buf[j] = jnp.where(row == b, oj, oh_buf[j])

            @_when(b == B - 1)
            def _():
                @_when(hg == 0)
                def _():
                    wait(wo_buf.at[:, pl.ds(0, (G - 1) * Dh), :], S_WO)
                oh0_buf[hg] = oh_buf[G - 1].astype(BF16)
                a = acc_buf[...]
                for j in range(G - 1):
                    a = a + jnp.dot(oh_buf[j].astype(BF16), wo_buf[hg, pl.ds(j * Dh, Dh), :],
                                    preferred_element_type=F32)
                acc_buf[...] = a

    for p in range(NW):
        k_part(p)
        issue_extras(p)
        if p + NS < NW:
            issue_head(p + NS)
        else:
            issue_pair(p + NS)

    def step(p, carry):
        v_part(p - NW)
        k_part(p)
        issue_extras(p)
        issue_pair(p + NS)

        @pl.when(p == MLP_STEP)
        def _():
            wait(w3_buf, S_W3)
            h1 = jax.lax.dot_general(xm_buf[...], w3_buf[...], NT, preferred_element_type=F32)
            h1 = jax.nn.gelu(h1, approximate=True)
            wait(w4_buf, S_W4)
            acc_buf[...] += jnp.dot(h1.astype(BF16), w4_buf[...], preferred_element_type=F32)
        return carry

    jax.lax.fori_loop(NW, NSTEP - NS, step, 0)

    for p in range(NSTEP - NS, NSTEP):
        v_part(p - NW)
        k_part(p)
        u = NSTEP - NW + 2 * (p - (NSTEP - NS))
        if u < NSTEP:
            issue_vv(u)
        if p == NSTEP - 1:
            issue_tail()
    for u in range(NSTEP - NW, NSTEP):
        v_part(u)

    a = acc_buf[...]
    h = 0
    for gi, n in enumerate(TAIL):
        wait(wo_buf.at[pl.ds(h, n), pl.ds((G - 1) * Dh, Dh), :], S_T + gi)
        for _ in range(n):
            a = a + jnp.dot(oh0_buf[h], wo_buf[h, pl.ds((G - 1) * Dh, Dh), :], preferred_element_type=F32)
            h += 1
    o_ref[...] = a[:B].astype(o_ref.dtype)


@jax.jit
def pallas_parallel_sum__sliding_block_cached__mixer_s_mlp__decode_kernel(
    A_x, A_k_cache, A_v_cache, A_wq, A_wo, B_x, B_w1, B_w2, B_w3, B_w4,
):
    B, Sq, D = A_x.shape
    _, H, S, Dh = A_k_cache.shape
    F = B_w3.shape[1]
    W = min(4096, max(256, S // 4))
    WB = W // G
    NHG = H // G
    assert Sq == 1 and B <= 8 and A_wq.shape == (D, H * Dh) and H % G == 0
    assert W % (G * R) == 0 and F % WR == 0 and 8 + F // WR <= MLP_STEP < NHG * B * G - NS
    assert 2 * (NS - 1) >= G
    kern = functools.partial(_kernel, B=B, H=H, S=S, W=W, Dh=Dh, D=D, F=F)
    out = pl.pallas_call(
        kern,
        in_specs=[pl.BlockSpec(memory_space=pl.ANY)] * 7,
        out_specs=pl.BlockSpec(memory_space=pltpu.VMEM),
        out_shape=jax.ShapeDtypeStruct((B, D), A_x.dtype),
        scratch_shapes=[
            pltpu.VMEM((B, D), BF16),
            pltpu.VMEM((4, D // 4, H * Dh), BF16),
            pltpu.VMEM((NHG, G * Dh, D), BF16),
            pltpu.VMEM((F, D), BF16),
            pltpu.VMEM((F, D), BF16),
            pltpu.VMEM((NS, G, WB, Dh), BF16),
            pltpu.VMEM((NS + G, G, WB, Dh), BF16),
            pltpu.VMEM((8, D), BF16),
            pltpu.VMEM((8, D), BF16),
            pltpu.VMEM((8, G * Dh), F32),
            pltpu.VMEM((8, Dh), BF16),
            pltpu.VMEM((G, 8, WB), F32),
            pltpu.VMEM((G, 8, WB), BF16),
            pltpu.VMEM((8, Dh), F32),
            pltpu.VMEM((8, Dh), F32),
            pltpu.VMEM((G, 8, Dh), F32),
            pltpu.VMEM((NHG, 8, Dh), BF16),
            pltpu.VMEM((8, D), F32),
            pltpu.SemaphoreType.DMA((4 + NHG + 2 * NS + G + len(TAIL),)),
        ],
        compiler_params=pltpu.CompilerParams(vmem_limit_bytes=64 * 1024 * 1024,
                                             disable_semaphore_checks=True),
    )(A_x.reshape(B, D), A_k_cache, A_v_cache, A_wq.reshape(4, D // 4, H * Dh),
      A_wo.reshape(NHG, G * Dh, D), B_w3.T, B_w4)
    return out.reshape(B, Sq, D)
```
